```python
import jax
import jax.numpy as jnp

def _softmax(x, axis=-1):
    return jax.nn.softmax(x, axis=axis)
def _gelu(x):
    return jax.nn.gelu(x, approximate=True)
def _silu(x):
    return jax.nn.silu(x)
def _sigmoid(x):
    return jax.nn.sigmoid(x)
def _layernorm(x, axis=-1, eps=1e-5):
    m = jnp.mean(x, axis=axis, keepdims=True)
    v = jnp.var(x, axis=axis, keepdims=True)
    return (x - m) / jnp.sqrt(v + eps)
def _scatter_add(tgt, idx, src, axis=0):
    return tgt.at[idx].add(src)
def _segment_sum(src, seg, n):
    return jax.ops.segment_sum(src, seg, n)
class _Rng:
    def __init__(self, key):
        self._k = key
    def _next(self):
        self._k, sub = jax.random.split(self._k)
        return sub
    def normal(self, shape):
        return jax.random.normal(self._next(), shape, dtype=jnp.bfloat16)
    def randint(self, lo, hi, shape):
        return jax.random.randint(self._next(), shape, lo, hi, dtype=jnp.int32)
    def uniform(self, shape, lo=0.0, hi=1.0):
        return jax.random.uniform(self._next(), shape, jnp.bfloat16, lo, hi)
    def permutation(self, n):
        return jax.random.permutation(self._next(), n)


kernel_name = 'sequential_preLN__linear_attn_block__moe_arch_mod__prompt'

def setup_inputs():
    _rng = _Rng(jax.random.key(int.from_bytes(__import__("os").urandom(4), "little")))
    _w = (lambda a: (lambda t: t.astype(jnp.bfloat16) if jnp.issubdtype(t.dtype, jnp.floating) else t)(jnp.asarray(a)))
    def _A_setup():
        B, S, D = 1, 2048, 1024
        return {
            "x": _w((lambda *s: _rng.normal(s) * 0.05)(B, S, D)),
            "wqkv": _w((lambda *s: _rng.normal(s) * 0.05)(D, 3 * D)),
            "wo": _w((lambda *s: _rng.normal(s) * 0.05)(D, D)),
        }
    _A_in = _A_setup()

    def _B_setup():
        B, S, D, F, C = 1, 2048, 1024, 3584, 2
        return {
            "x": _w((lambda *s: _rng.normal(s) * 0.05)(B, S, D)),
            "w_r": _w((lambda *s: _rng.normal(s) * 0.05)(D)),
            "w_gate": _w((lambda *s: _rng.normal(s) * 0.05)(D, F)),
            "w_up": _w((lambda *s: _rng.normal(s) * 0.05)(D, F)),
            "w_down": _w((lambda *s: _rng.normal(s) * 0.05)(F, D)),
        }
    _B_in = _B_setup()

    return {
        "A_x": _A_in["x"],
        "A_wqkv": _A_in["wqkv"],
        "A_wo": _A_in["wo"],
        "B_x": _B_in["x"],
        "B_w_r": _B_in["w_r"],
        "B_w_gate": _B_in["w_gate"],
        "B_w_up": _B_in["w_up"],
        "B_w_down": _B_in["w_down"],
    }

def reference(A_x, A_wqkv, A_wo, B_x, B_w_r, B_w_gate, B_w_up, B_w_down):
    def _A_ref(x, wqkv, wo):
        B, S, D = x.shape
        H = 32; Dh = D // H
        qkv = (lambda x, *d: x.transpose(*d))((x @ wqkv).reshape(B, S, 3, H, Dh), 2, 0, 3, 1, 4)
        q, k, v = qkv[0], qkv[1], qkv[2]
        phi = lambda t: jnp.where(t > 0, t + 1, jnp.exp(t)) + 1e-6
        pq, pk = phi(q), phi(k)
        kv = jnp.einsum("bhsd,bhse->bhde", pk, v)
        z = jnp.einsum("bhsd->bhd", pk)
        num = jnp.einsum("bhqd,bhde->bhqe", pq, kv)
        den = jnp.einsum("bhqd,bhd->bhq", pq, z)[..., None] + 1e-6
        o = num / den
        return (lambda x, *d: x.transpose(*d))(o, 0, 2, 1, 3).reshape(B, S, D) @ wo

    def _B_ref(x, w_r, w_gate, w_up, w_down):
        B, S, D = x.shape
        C = 2
        r = x @ w_r
        idx = jnp.argsort(-r, axis=-1)[:, :C]
        idx_e = jnp.repeat(idx.reshape(B, C, 1), D, axis=2)
        x_sel = jnp.take_along_axis(x, idx_e, axis=1)
        g = _silu(x_sel @ w_gate)
        u = x_sel @ w_up
        y = (g * u) @ w_down
        r_sel = _sigmoid(jnp.take_along_axis(r, idx, axis=1))
        y = y * r_sel.reshape(B, C, 1)
        b_off = (jnp.arange(B) * S).reshape(B, 1)
        flat_idx = (idx + b_off).reshape(B * C)
        zero = (x * 0.0).reshape(B * S, D)
        upd = _scatter_add(zero, flat_idx, y.reshape(B * C, D), axis=0)
        return x + upd.reshape(B, S, D)

    x = A_x
    h = x + _A_ref(_layernorm(x, axis=-1), A_wqkv, A_wo)
    h2 = h + _B_ref(_layernorm(h, axis=-1), B_w_r, B_w_gate, B_w_up, B_w_down)
    return h2
```

```python
import jax
import jax.numpy as jnp
from jax import lax
import jax.experimental.pallas as pl
import jax.experimental.pallas.tpu as pltpu

S, D, H, DH, F = 2048, 1024, 32, 32, 3584
TS = 512
TM = 256
NX = S // TM
RB = 256
CH = 16
BF = jnp.bfloat16
F32 = jnp.float32


def _phi(t):
    return jnp.where(t > 0, t + 1.0, jnp.exp(t)) + 1e-6


def _ln(x):
    m = jnp.mean(x, axis=-1, keepdims=True)
    c = x - m
    v = jnp.mean(c * c, axis=-1, keepdims=True)
    return c * lax.rsqrt(v + 1e-5)


def _nt(a, b):
    return lax.dot_general(a, b, (((1,), (1,)), ((), ())), preferred_element_type=F32)


def _nn(a, b):
    return jnp.dot(a, b, preferred_element_type=F32)


def _kernel(x_hbm, wqkv_hbm, wo_hbm, wr_hbm, wg_hbm, wu_hbm, wd_hbm, out_hbm,
            x_v, xn_v, hs, pqs, pk_v, wq_v, wk_v, wv_v, wkt_v, wqt_v, wo_v, wr_v,
            wg_v, wu_v, wd_v, t_acc, z_acc, m_v, sem_x, sem_w, sem_o, sem_p, sem_k):
    o_v = x_v
    hn_v = xn_v

    def rows_(r, n):
        return pl.ds(pl.multiple_of(r, CH), n) if not isinstance(r, int) else pl.ds(r, n)

    def x_copy(i):
        return pltpu.make_async_copy(x_hbm.at[pl.ds(i * TM, TM)], x_v.at[pl.ds(i * TM, TM)], sem_x.at[i])

    def o_copy(i):
        return pltpu.make_async_copy(o_v.at[pl.ds(i * TM, TM)], out_hbm.at[pl.ds(i * TM, TM)], sem_o.at[i])

    def wk_copy(c):
        return pltpu.make_async_copy(wqkv_hbm.at[:, pl.ds(D + c * RB, RB)], wk_v.at[:, pl.ds(c * RB, RB)], sem_k.at[c])

    c_wq = pltpu.make_async_copy(wqkv_hbm.at[:, pl.ds(0, D)], wq_v, sem_w.at[1])
    c_wv = pltpu.make_async_copy(wqkv_hbm.at[:, pl.ds(2 * D, D)], wv_v, sem_w.at[2])
    c_wo = pltpu.make_async_copy(wo_hbm, wo_v, sem_w.at[3])
    c_wr = pltpu.make_async_copy(wr_hbm, wr_v, sem_w.at[4])
    c_wg = pltpu.make_async_copy(wg_hbm, wg_v, sem_w.at[5])
    c_wu = pltpu.make_async_copy(wu_hbm, wu_v, sem_w.at[6])
    c_wd = pltpu.make_async_copy(wd_hbm, wd_v, sem_w.at[7])
    NB = D // RB

    x_copy(0).start()
    wk_copy(0).start()
    x_copy(1).start()
    for c in range(1, NB):
        wk_copy(c).start()

    def ln_rows(r0, n):
        for r in range(r0, r0 + n, CH):
            xn_v[r:r + CH, :] = _ln(x_v[r:r + CH, :].astype(F32)).astype(BF)

    def wt_block(src, dst, c):
        for j in range(RB // 128):
            cc = c * RB + j * 128
            dst[cc:cc + 128, :] = src[:, cc:cc + 128].T

    t_acc[...] = jnp.zeros_like(t_acc)
    z_acc[...] = jnp.zeros_like(z_acc)
    x_copy(0).wait()
    ln_rows(0, TM)
    x_copy(1).wait()
    ln_rows(TM, TM)

    NT1 = S // TS
    for i in range(NT1):
        r0 = i * TS
        if 0 < i < NT1 - 1:
            x_copy(2 * i + 2).wait(); x_copy(2 * i + 3).wait()
        if i == 1:
            c_wg.start(); c_wu.start(); c_wd.start()
        if i == NT1 - 1:
            c_wq.wait()
        lnp = TS // (2 * NB)
        for c in range(NB):
            if i == 0:
                wk_copy(c).wait()
                if c == 1:
                    x_copy(2).start(); x_copy(3).start()
                if c == NB - 1:
                    for j in range(4, NX):
                        x_copy(j).start()
                wt_block(wk_v, wkt_v, c)
            sl = slice(c * RB, (c + 1) * RB)
            pk = _phi(_nt(wkt_v[sl, :], xn_v[r0:r0 + TS, :])).astype(BF)
            pk_v[sl, :] = pk
            pkf = pk.astype(F32)
            zs = pkf[:, 0:128]
            for t in range(1, TS // 128):
                zs = zs + pkf[:, t * 128:(t + 1) * 128]
            z_acc[sl, :] += zs
            if 0 < i < NT1 - 1:
                ln_rows(r0 + TS + c * lnp, lnp)
            if i == NT1 - 1:
                wt_block(wq_v, wqt_v, c)
        if i == 0:
            x_copy(2).wait(); x_copy(3).wait()
            c_wq.start(); c_wv.start(); c_wo.start(); c_wr.start()
        for c in range(NB):
            sl = slice(c * RB, (c + 1) * RB)
            t_acc[:, sl] += _nn(pk_v[...], xn_v[r0:r0 + TS, sl])
            if i == 0:
                ln_rows(r0 + TS + c * 2 * lnp, 2 * lnp)
            elif i < NT1 - 1:
                ln_rows(r0 + TS + (NB + c) * lnp, lnp)

    c_wv.wait(); c_wo.wait(); c_wr.wait()

    for c in range(NB):
        sl = slice(c * RB, (c + 1) * RB)
        z_acc[sl, :] = jnp.broadcast_to(jnp.sum(z_acc[sl, :], axis=1, keepdims=True), (RB, 128))
    ri = lax.broadcasted_iota(jnp.int32, (128, 128), 0) // DH
    ci = lax.broadcasted_iota(jnp.int32, (128, 128), 1) // DH
    msk = ri == ci

    def m_group(g):
        sl = slice(g * 128, (g + 1) * 128)
        kv = _nn(t_acc[sl, :].astype(BF), wv_v[:, sl])
        kv = jnp.where(msk, kv, 0.0).astype(BF)
        m_v[sl, :] = _nn(kv, wo_v[sl, :]).astype(BF)

    def q_piece(i, c):
        r0 = i * TM
        sl = slice(c * RB, (c + 1) * RB)
        pq = _phi(_nt(wqt_v[sl, :], xn_v[rows_(r0, TM), :]))
        zb = z_acc[sl, :].reshape(RB // DH, DH, 128)
        for t in range(TM // 128):
            p3 = pq[:, t * 128:(t + 1) * 128].reshape(RB // DH, DH, 128)
            den = jnp.sum(p3 * zb, axis=1, keepdims=True) + 1e-6
            pn = (p3 / den).reshape(RB, 128).astype(BF)
            pqs[i % 2, t * 128:(t + 1) * 128, sl] = pn.T

    def a_piece(i, c):
        r0 = i * TM
        sl = slice(c * RB, (c + 1) * RB)
        hs[i % 2, :, sl] = x_v[rows_(r0, TM), sl].astype(F32) + _nn(pqs[i % 2], m_v[:, sl])

    def post_rows(i, q0, n, carry):
        m1, i1, m2, i2 = carry
        for q in range(q0, q0 + n, CH):
            r0 = i * TM + q
            h = hs[i % 2, q:q + CH, :]
            hn = _ln(h)
            o_v[rows_(r0, CH), :] = (h + hn).astype(BF)
            hnb = hn.astype(BF)
            hn_v[rows_(r0, CH), :] = hnb
            r = jnp.sum(hnb.astype(F32) * wr_v[...].astype(F32), axis=1, keepdims=True)
            for b in range(CH // 8):
                rv = jnp.broadcast_to(r[b * 8:(b + 1) * 8], (8, 128))
                iv = lax.broadcasted_iota(jnp.int32, (8, 128), 0) + (r0 + b * 8)
                g1 = rv > m1
                g2 = rv > m2
                m2 = jnp.where(g1, m1, jnp.where(g2, rv, m2))
                i2 = jnp.where(g1, i1, jnp.where(g2, iv, i2))
                m1 = jnp.where(g1, rv, m1)
                i1 = jnp.where(g1, iv, i1)
        return m1, i1, m2, i2

    for g in range(8):
        m_group(g)
        if g % 2 == 1:
            q_piece(0, g // 2)
    neg = jnp.full((8, 128), -jnp.inf, F32)
    zi = jnp.zeros((8, 128), jnp.int32)
    carry = (neg, zi, neg, zi)
    pp = TM // (2 * NB)
    for c in range(NB):
        q_piece(1, c)
    for c in range(NB):
        a_piece(0, c)

    def body(i, carry):
        for c in range(NB):
            q_piece(i + 1, c)
            carry = post_rows(i - 1, c * pp, pp, carry)
        for c in range(NB):
            a_piece(i, c)
            carry = post_rows(i - 1, (NB + c) * pp, pp, carry)
        o_copy(i - 1).start()
        return carry
    carry = lax.fori_loop(1, NX - 1, body, carry)
    for c in range(NB):
        a_piece(NX - 1, c)
        carry = post_rows(NX - 2, c * 2 * pp, 2 * pp, carry)
    o_copy(NX - 2).start()
    m1, i1, m2, i2 = post_rows(NX - 1, 0, TM, carry)
    o_copy(NX - 1).start()

    big = jnp.int32(1 << 30)
    v1 = jnp.max(m1)
    s1 = jnp.min(jnp.where(m1 == v1, i1, big))
    mm = jnp.where(i1 == s1, m2, m1)
    ii = jnp.where(i1 == s1, i2, i1)
    v2 = jnp.max(mm)
    s2 = jnp.min(jnp.where(mm == v2, ii, big))
    s1 = jnp.clip(s1, 0, S - 1)
    s2 = jnp.clip(s2, 0, S - 1)
    b1 = pl.multiple_of((s1 // 16) * 16, 16)
    b2 = pl.multiple_of((s2 // 16) * 16, 16)
    rows = lax.broadcasted_iota(jnp.int32, (16, D), 0)
    xa = jnp.sum(jnp.where(rows == s1 - b1, hn_v[pl.ds(b1, 16), :].astype(F32), 0.0), axis=0, keepdims=True)
    xb = jnp.sum(jnp.where(rows == s2 - b2, hn_v[pl.ds(b2, 16), :].astype(F32), 0.0), axis=0, keepdims=True)
    xs = jnp.where(rows == 0, xa, jnp.where(rows == 1, xb, 0.0)).astype(BF)
    c_wg.wait(); c_wu.wait(); c_wd.wait()
    y = jnp.zeros((16, D), F32)
    FB = 512
    for f in range(0, F, FB):
        g = _nn(xs, wg_v[:, f:f + FB])
        u = _nn(xs, wu_v[:, f:f + FB])
        a = (g * jax.nn.sigmoid(g) * u).astype(BF)
        y = y + _nn(a, wd_v[f:f + FB, :])
    rsel = jnp.where(rows[:, 0:1] == 0, v1, v2)
    y = y * jax.nn.sigmoid(rsel)
    for i in range(NX):
        o_copy(i).wait()
    o_v[pl.ds(b1, 16), :] = (o_v[pl.ds(b1, 16), :].astype(F32) + jnp.where(rows == s1 - b1, y[0:1], 0.0)).astype(BF)
    o_v[pl.ds(b2, 16), :] = (o_v[pl.ds(b2, 16), :].astype(F32) + jnp.where(rows == s2 - b2, y[1:2], 0.0)).astype(BF)
    p1c = pltpu.make_async_copy(o_v.at[pl.ds(b1, 16)], out_hbm.at[pl.ds(b1, 16)], sem_p.at[0])
    p2c = pltpu.make_async_copy(o_v.at[pl.ds(b2, 16)], out_hbm.at[pl.ds(b2, 16)], sem_p.at[1])
    p1c.start()

    @pl.when(b1 != b2)
    def _():
        p2c.start()
        p2c.wait()
    p1c.wait()


@jax.jit
def pallas_sequential_preLN__linear_attn_block__moe_arch_mod__prompt_kernel(
        A_x, A_wqkv, A_wo, B_x, B_w_r, B_w_gate, B_w_up, B_w_down):
    any_ = pl.BlockSpec(memory_space=pl.ANY)
    V = pltpu.VMEM
    DMA = pltpu.SemaphoreType.DMA
    out = pl.pallas_call(
        _kernel,
        in_specs=[any_] * 7,
        out_specs=any_,
        out_shape=jax.ShapeDtypeStruct((S, D), BF),
        scratch_shapes=[
            V((S, D), BF), V((S, D), BF),
            V((2, TM, D), F32), V((2, TM, D), BF), V((D, TS), BF),
            V((D, D), BF), V((D, D), BF), V((D, D), BF), V((D, D), BF), V((D, D), BF), V((D, D), BF), V((1, D), BF),
            V((D, F), BF), V((D, F), BF), V((F, D), BF),
            V((D, D), F32), V((D, 128), F32), V((D, D), BF),
            DMA((NX,)), DMA((8,)), DMA((NX,)), DMA((2,)), DMA((D // RB,)),
        ],
        compiler_params=pltpu.CompilerParams(vmem_limit_bytes=110 * 2**20),
    )(A_x.reshape(S, D), A_wqkv, A_wo, B_w_r.reshape(1, D), B_w_gate, B_w_up, B_w_down)
    return out.reshape(A_x.shape)
```

```python
import jax
import jax.numpy as jnp
from jax import lax
import jax.experimental.pallas as pl
import jax.experimental.pallas.tpu as pltpu

S, D, H, DH, F = 2048, 1024, 32, 32, 3584
TS = 512
TM = 256
NX = S // TM
RB = 256
CH = 16
BF = jnp.bfloat16
F32 = jnp.float32


def _phi(t):
    return jnp.where(t > 0, t + 1.0, jnp.exp(t)) + 1e-6


def _ln(x):
    m = jnp.mean(x, axis=-1, keepdims=True)
    c = x - m
    v = jnp.mean(c * c, axis=-1, keepdims=True)
    return c * lax.rsqrt(v + 1e-5)


def _nt(a, b):
    return lax.dot_general(a, b, (((1,), (1,)), ((), ())), preferred_element_type=F32)


def _nn(a, b):
    return jnp.dot(a, b, preferred_element_type=F32)


def _kernel(x_hbm, wqkv_hbm, wo_hbm, wr_hbm, wg_hbm, wu_hbm, wd_hbm, out_hbm,
            x_v, xn_v, hn_v, hs, pq0, pq1, pk_v, wq_v, wk_v, wv_v, wkt_v, wqt_v, wo_v, wr_v,
            wg_v, wu_v, wd_v, t_acc, z_acc, m_v, sem_x, sem_w, sem_o, sem_p, sem_k):
    pqs = [pq0, pq1]
    o_v = x_v

    def rows_(r, n):
        return pl.ds(pl.multiple_of(r, CH), n) if not isinstance(r, int) else pl.ds(r, n)

    def x_copy(i):
        return pltpu.make_async_copy(x_hbm.at[pl.ds(i * TM, TM)], x_v.at[pl.ds(i * TM, TM)], sem_x.at[i])

    def o_copy(i):
        return pltpu.make_async_copy(o_v.at[pl.ds(i * TM, TM)], out_hbm.at[pl.ds(i * TM, TM)], sem_o.at[i])

    def wk_copy(c):
        return pltpu.make_async_copy(wqkv_hbm.at[:, pl.ds(D + c * RB, RB)], wk_v.at[:, pl.ds(c * RB, RB)], sem_k.at[c])

    c_wq = pltpu.make_async_copy(wqkv_hbm.at[:, pl.ds(0, D)], wq_v, sem_w.at[1])
    c_wv = pltpu.make_async_copy(wqkv_hbm.at[:, pl.ds(2 * D, D)], wv_v, sem_w.at[2])
    c_wo = pltpu.make_async_copy(wo_hbm, wo_v, sem_w.at[3])
    c_wr = pltpu.make_async_copy(wr_hbm, wr_v, sem_w.at[4])
    c_wg = pltpu.make_async_copy(wg_hbm, wg_v, sem_w.at[5])
    c_wu = pltpu.make_async_copy(wu_hbm, wu_v, sem_w.at[6])
    c_wd = pltpu.make_async_copy(wd_hbm, wd_v, sem_w.at[7])
    NB = D // RB

    x_copy(0).start()
    wk_copy(0).start()
    x_copy(1).start()
    for c in range(1, NB):
        wk_copy(c).start()

    def ln_rows(r0, n):
        for r in range(r0, r0 + n, CH):
            xn_v[r:r + CH, :] = _ln(x_v[r:r + CH, :].astype(F32)).astype(BF)

    def wt_block(src, dst, c):
        for j in range(RB // 128):
            cc = c * RB + j * 128
            dst[cc:cc + 128, :] = src[:, cc:cc + 128].T

    x_copy(0).wait()
    ln_rows(0, TM)

    def k_piece(r0, n, t0, c, first):
        sl = slice(c * RB, (c + 1) * RB)
        pk = _phi(_nt(wkt_v[sl, :], xn_v[r0 + t0:r0 + t0 + n, :])).astype(BF)
        pk_v[sl, t0:t0 + n] = pk
        pkf = pk.astype(F32)
        zs = pkf[:, 0:128]
        for t in range(1, n // 128):
            zs = zs + pkf[:, t * 128:(t + 1) * 128]
        z_acc[sl, :] = zs if first else z_acc[sl, :] + zs

    NT1 = S // TS
    for i in range(NT1):
        r0 = i * TS
        if i == 0:
            for c in range(NB):
                wk_copy(c).wait()
                if c == 1:
                    x_copy(1).wait()
                    x_copy(2).start(); x_copy(3).start()
                if c == NB - 1:
                    for j in range(4, NX):
                        x_copy(j).start()
                wt_block(wk_v, wkt_v, c)
                k_piece(0, TM, 0, c, True)
                if c >= 1:
                    ln_rows(TM + (c - 1) * 96, 96 if c < 3 else 64)
            for c in range(NB):
                k_piece(0, TM, TM, c, False)
            c_wq.start(); c_wv.start(); c_wo.start(); c_wr.start()
        if i < NT1 - 1:
            x_copy(2 * i + 2).wait(); x_copy(2 * i + 3).wait()
        if i == 1:
            c_wg.start(); c_wu.start(); c_wd.start()
        if i == NT1 - 1:
            c_wq.wait()
        if i > 0:
            for c in range(NB):
                k_piece(r0, TS, 0, c, False)
                if i < NT1 - 1:
                    ln_rows(r0 + TS + c * 64, 64)
                else:
                    wt_block(wq_v, wqt_v, c)
        for c in range(NB):
            sl = slice(c * RB, (c + 1) * RB)
            if i == 0:
                ln_rows(TS + c * 128, 128)
            elif i < NT1 - 1:
                ln_rows(r0 + TS + 256 + c * 64, 64)
            d = _nn(pk_v[...], xn_v[r0:r0 + TS, sl])
            t_acc[:, sl] = d if i == 0 else t_acc[:, sl] + d

    c_wv.wait(); c_wo.wait(); c_wr.wait()

    for c in range(NB):
        sl = slice(c * RB, (c + 1) * RB)
        z_acc[sl, :] = jnp.broadcast_to(jnp.sum(z_acc[sl, :], axis=1, keepdims=True), (RB, 128))
    ri = lax.broadcasted_iota(jnp.int32, (128, 128), 0) // DH
    ci = lax.broadcasted_iota(jnp.int32, (128, 128), 1) // DH
    msk = ri == ci

    wr = wr_v[...].astype(F32).reshape(1, D)

    def m_group(g):
        sl = slice(g * 128, (g + 1) * 128)
        kv = _nn(t_acc[sl, :].astype(BF), wv_v[:, sl])
        kv = jnp.where(msk, kv, 0.0).astype(BF)
        m_v[sl, :] = _nn(kv, wo_v[sl, :]).astype(BF)

    def q_piece(i, c, p):
        r0 = i * TM
        sl = slice(c * RB, (c + 1) * RB)
        pq = _phi(_nt(wqt_v[sl, :], xn_v[rows_(r0, TM), :]))
        zb = z_acc[sl, :].reshape(RB // DH, DH, 128)
        for t in range(TM // 128):
            p3 = pq[:, t * 128:(t + 1) * 128].reshape(RB // DH, DH, 128)
            den = jnp.sum(p3 * zb, axis=1, keepdims=True) + 1e-6
            pn = (p3 / den).reshape(RB, 128).astype(BF)
            pqs[p][t * 128:(t + 1) * 128, sl] = pn.T

    def a_piece(i, c, p):
        r0 = i * TM
        sl = slice(c * RB, (c + 1) * RB)
        hs[p, :, sl] = x_v[rows_(r0, TM), sl].astype(F32) + _nn(pqs[p][...], m_v[:, sl])

    def post_rows(i, p, q0, n, carry):
        m1, i1, m2, i2 = carry
        for q in range(q0, q0 + n, CH):
            r0 = i * TM + q
            h = hs[p, q:q + CH, :]
            hn = _ln(h)
            o_v[rows_(r0, CH), :] = (h + hn).astype(BF)
            hnb = hn.astype(BF)
            hn_v[rows_(r0, CH), :] = hnb
            r = jnp.sum(hnb.astype(F32) * wr, axis=1, keepdims=True)
            for b in range(CH // 8):
                rv = jnp.broadcast_to(r[b * 8:(b + 1) * 8], (8, 128))
                iv = lax.broadcasted_iota(jnp.int32, (8, 128), 0) + (r0 + b * 8)
                g1 = rv > m1
                g2 = rv > m2
                m2 = jnp.where(g1, m1, jnp.where(g2, rv, m2))
                i2 = jnp.where(g1, i1, jnp.where(g2, iv, i2))
                m1 = jnp.where(g1, rv, m1)
                i1 = jnp.where(g1, iv, i1)
        return m1, i1, m2, i2

    for g in range(8):
        m_group(g)
        if g % 2 == 1:
            q_piece(0, g // 2, 0)
    neg = jnp.full((8, 128), -jnp.inf, F32)
    zi = jnp.zeros((8, 128), jnp.int32)
    carry = (neg, zi, neg, zi)
    pp = TM // (2 * NB)
    for c in range(NB):
        q_piece(1, c, 1)
    for c in range(NB):
        a_piece(0, c, 0)

    def body(j, carry):
        for p in (1, 0):
            i = 2 * j + (2 - p)
            for c in range(NB):
                q_piece(i + 1, c, 1 - p)
                carry = post_rows(i - 1, 1 - p, c * 48, 48, carry)
            for c in range(NB):
                a_piece(i, c, p)
                if c < 2:
                    carry = post_rows(i - 1, 1 - p, 192 + c * 32, 32, carry)
        o_copy(2 * j).start()
        o_copy(2 * j + 1).start()
        return carry
    carry = lax.fori_loop(0, (NX - 2) // 2, body, carry)
    for c in range(NB):
        carry = post_rows(NX - 2, 0, c * 2 * pp, 2 * pp, carry)
        a_piece(NX - 1, c, 1)
    o_copy(NX - 2).start()
    m1, i1, m2, i2 = post_rows(NX - 1, 1, 0, TM, carry)
    o_copy(NX - 1).start()

    big = jnp.int32(1 << 30)
    v1 = jnp.max(m1)
    s1 = jnp.min(jnp.where(m1 == v1, i1, big))
    mm = jnp.where(i1 == s1, m2, m1)
    ii = jnp.where(i1 == s1, i2, i1)
    v2 = jnp.max(mm)
    s2 = jnp.min(jnp.where(mm == v2, ii, big))
    s1 = jnp.clip(s1, 0, S - 1)
    s2 = jnp.clip(s2, 0, S - 1)
    b1 = pl.multiple_of((s1 // 16) * 16, 16)
    b2 = pl.multiple_of((s2 // 16) * 16, 16)
    rows = lax.broadcasted_iota(jnp.int32, (16, D), 0)
    xa = jnp.sum(jnp.where(rows == s1 - b1, hn_v[pl.ds(b1, 16), :].astype(F32), 0.0), axis=0, keepdims=True)
    xb = jnp.sum(jnp.where(rows == s2 - b2, hn_v[pl.ds(b2, 16), :].astype(F32), 0.0), axis=0, keepdims=True)
    xs = jnp.where(rows == 0, xa, jnp.where(rows == 1, xb, 0.0)).astype(BF)
    c_wg.wait(); c_wu.wait(); c_wd.wait()
    y = jnp.zeros((16, D), F32)
    FB = 896
    for f in range(0, F, FB):
        g = _nn(xs, wg_v[:, f:f + FB])
        u = _nn(xs, wu_v[:, f:f + FB])
        a = (g * jax.nn.sigmoid(g) * u).astype(BF)
        y = y + _nn(a, wd_v[f:f + FB, :])
    rsel = jnp.where(rows[:, 0:1] == 0, v1, v2)
    y = y * jax.nn.sigmoid(rsel)
    for i in range(NX):
        o_copy(i).wait()
    o_v[pl.ds(b1, 16), :] = (o_v[pl.ds(b1, 16), :].astype(F32) + jnp.where(rows == s1 - b1, y[0:1], 0.0)).astype(BF)
    o_v[pl.ds(b2, 16), :] = (o_v[pl.ds(b2, 16), :].astype(F32) + jnp.where(rows == s2 - b2, y[1:2], 0.0)).astype(BF)
    p1c = pltpu.make_async_copy(o_v.at[pl.ds(b1, 16)], out_hbm.at[pl.ds(b1, 16)], sem_p.at[0])
    p2c = pltpu.make_async_copy(o_v.at[pl.ds(b2, 16)], out_hbm.at[pl.ds(b2, 16)], sem_p.at[1])
    p1c.start()

    @pl.when(b1 != b2)
    def _():
        p2c.start()
        p2c.wait()
    p1c.wait()


@jax.jit
def pallas_sequential_preLN__linear_attn_block__moe_arch_mod__prompt_kernel(
        A_x, A_wqkv, A_wo, B_x, B_w_r, B_w_gate, B_w_up, B_w_down):
    any_ = pl.BlockSpec(memory_space=pl.ANY)
    V = pltpu.VMEM
    DMA = pltpu.SemaphoreType.DMA
    out = pl.pallas_call(
        _kernel,
        in_specs=[any_] * 7,
        out_specs=any_,
        out_shape=jax.ShapeDtypeStruct((S, D), BF),
        scratch_shapes=[
            V((S, D), BF), V((S, D), BF), V((S, D), BF),
            V((2, TM, D), F32), V((TM, D), BF), V((TM, D), BF), V((D, TS), BF),
            V((D, D), BF), V((D, D), BF), V((D, D), BF), V((D, D), BF), V((D, D), BF), V((D, D), BF), V((D,), BF),
            V((D, F), BF), V((D, F), BF), V((F, D), BF),
            V((D, D), F32), V((D, 128), F32), V((D, D), BF),
            DMA((NX,)), DMA((8,)), DMA((NX,)), DMA((2,)), DMA((D // RB,)),
        ],
        compiler_params=pltpu.CompilerParams(vmem_limit_bytes=110 * 2**20, flags={'XLA_TPU_EVENLY_DISTRIBUTE_CRITICAL_NODES': True}),
    )(A_x.reshape(S, D), A_wqkv, A_wo, B_w_r, B_w_gate, B_w_up, B_w_down)
    return out.reshape(A_x.shape)
```
